```python
import jax
import jax.numpy as jnp

def _softmax(x, axis=-1):
    return jax.nn.softmax(x, axis=axis)

def _gelu(x):
    return jax.nn.gelu(x, approximate=True)

def _silu(x):
    return jax.nn.silu(x)

def _sigmoid(x):
    return jax.nn.sigmoid(x)

def _layernorm(x, axis=-1, eps=1e-05):
    m = jnp.mean(x, axis=axis, keepdims=True)
    v = jnp.var(x, axis=axis, keepdims=True)
    return (x - m) / jnp.sqrt(v + eps)

def _scatter_add(tgt, idx, src, axis=0):
    return tgt.at[idx].add(src)

def _segment_sum(src, seg, n):
    return jax.ops.segment_sum(src, seg, n)

class _Rng:

    def __init__(self, key):
        self._k = key

    def _next(self):
        self._k, sub = jax.random.split(self._k)
        return sub

    def normal(self, shape):
        return jax.random.normal(self._next(), shape, dtype=jnp.bfloat16)

    def randint(self, lo, hi, shape):
        return jax.random.randint(self._next(), shape, lo, hi, dtype=jnp.int32)

    def uniform(self, shape, lo=0.0, hi=1.0):
        return jax.random.uniform(self._next(), shape, jnp.bfloat16, lo, hi)

    def permutation(self, n):
        return jax.random.permutation(self._next(), n)
kernel_name = 'interleave_layers__sliding_local_dilated__mixer_gmlp__prompt'

def setup_inputs():
    _rng = _Rng(jax.random.key(int.from_bytes(__import__("os").urandom(4), "little")))
    _w = lambda a: (lambda t: t.astype(jnp.bfloat16) if jnp.issubdtype(t.dtype, jnp.floating) else t)(jnp.asarray(a))

    def _A_setup():
        B, S, D = (1, 2048, 576)
        return {'x': _w((lambda *s: _rng.normal(s) * 0.05)(B, S, D)), 'wqkv': _w((lambda *s: _rng.normal(s) * 0.05)(D, 3 * D)), 'wo': _w((lambda *s: _rng.normal(s) * 0.05)(D, D))}
    _A_in = _A_setup()

    def _B_setup():
        B, S, D, F = (1, 2048, 576, 4608)
        Fh = F // 2
        return {'x': _w((lambda *s: _rng.normal(s) * 0.05)(B, S, D)), 'w_in': _w((lambda *s: _rng.normal(s) * 0.05)(D, 2 * Fh)), 'w_sp': _w(0.01 * (lambda *s: _rng.normal(s) * 0.05)(S, S)), 'b_sp': _w(1.0 + 0.01 * (lambda *s: _rng.normal(s) * 0.05)(S)), 'w_out': _w((lambda *s: _rng.normal(s) * 0.05)(Fh, D))}
    _B_in = _B_setup()
    return {'A_x': _A_in['x'], 'A_wqkv': _A_in['wqkv'], 'A_wo': _A_in['wo'], 'B_x': _B_in['x'], 'B_w_in': _B_in['w_in'], 'B_w_sp': _B_in['w_sp'], 'B_b_sp': _B_in['b_sp'], 'B_w_out': _B_in['w_out']}

def reference(A_x, A_wqkv, A_wo, B_x, B_w_in, B_w_sp, B_b_sp, B_w_out):

    def _A_ref(x, wqkv, wo):
        B, S, D = x.shape
        H = 32
        Dh = D // H
        W, dil = (8, 2)
        qkv = (lambda x, *d: x.transpose(*d))((x @ wqkv).reshape(B, S, 3, H, Dh), 2, 0, 3, 1, 4)
        q, k, v = (qkv[0], qkv[1], qkv[2])
        scale = Dh ** (-0.5)
        pos = jnp.arange(S)
        off = jnp.arange(W) * dil
        idx = pos[:, None] - off[None, :]
        mask = idx >= 0
        idx_c = jnp.where(mask, idx, 0).reshape(-1)
        kg = k[:, :, idx_c, :].reshape(B, H, S, W, Dh)
        vg = v[:, :, idx_c, :].reshape(B, H, S, W, Dh)
        logits = jnp.einsum('bhsd,bhswd->bhsw', q, kg) * scale
        logits = jnp.where(mask[None, None, :, :], logits, -1000000000.0)
        attn = _softmax(logits, axis=-1)
        o = jnp.einsum('bhsw,bhswd->bhsd', attn, vg)
        return (lambda x, *d: x.transpose(*d))(o, 0, 2, 1, 3).reshape(B, S, D) @ wo

    def _B_ref(x, w_in, w_sp, b_sp, w_out):
        B, S, D = x.shape
        F = w_in.shape[-1]
        Fh = F // 2
        z = _gelu(jnp.einsum('bsd,df->bsf', x, w_in))
        z1 = z[..., :Fh].copy()
        z2 = _layernorm(z[..., Fh:], axis=-1)
        g = jnp.einsum('ts,bsf->btf', w_sp, z2) + b_sp[None, :, None]
        return jnp.einsum('bsf,fd->bsd', z1 * g, w_out)
    x = A_x
    x = x + _A_ref(_layernorm(x, axis=-1), A_wqkv, A_wo)
    x = x + _B_ref(_layernorm(x, axis=-1), B_w_in, B_w_sp, B_b_sp, B_w_out)
    x = x + _A_ref(_layernorm(x, axis=-1), A_wqkv, A_wo)
    x = x + _B_ref(_layernorm(x, axis=-1), B_w_in, B_w_sp, B_b_sp, B_w_out)
    return x
```

```python
import math

import jax
import jax.numpy as jnp
from jax import lax
import jax.experimental.pallas as pl
import jax.experimental.pallas.tpu as pltpu

S, D, H, DH, W, DIL = 2048, 576, 32, 18, 8, 2
FH = 2304
TM = 256
HALO = 16
NT = S // TM
F32, BF16 = jnp.float32, jnp.bfloat16


def _mm(a, b):
    return jnp.dot(a, b, preferred_element_type=F32)


def _ln(x):
    m = jnp.mean(x, axis=-1, keepdims=True)
    c = x - m
    v = jnp.mean(c * c, axis=-1, keepdims=True)
    return c * lax.rsqrt(v + 1e-5)


def _gelu(x):
    k = math.sqrt(2.0 / math.pi)
    u = x * (k + (k * 0.044715) * (x * x))
    hx = 0.5 * x
    return hx + hx * jnp.tanh(u)


def _onehot(shape, src_axis, src_fn):
    s = lax.broadcasted_iota(jnp.int32, shape, src_axis)
    d = lax.broadcasted_iota(jnp.int32, shape, 1 - src_axis)
    return jnp.where(s == src_fn(d), 1.0, 0.0).astype(BF16)


def _kernel(x_hbm, wqkv_hbm, wo_hbm, win_hbm, wsp_hbm, b_ref, wout_hbm, o_hbm,
            x0, wqkv, wo, win, wsp, wout, wq_p, wo_p, xs, z1, z2a, z2b, kv, bias,
            obuf, sems, osem):
    cps = [pltpu.make_async_copy(s, d, sems.at[i]) for i, (s, d) in enumerate(
        [(wqkv_hbm, wqkv), (x_hbm, x0), (wo_hbm, wo), (win_hbm, win),
         (wsp_hbm, wsp), (wout_hbm, wout)])]
    for c in cps:
        c.start()

    hd = lambda j: (j & 31) * DH + (j >> 5)
    cps[0].wait()
    wq_p[:, 0:512] = _mm(wqkv[:, 0:640], _onehot((640, 512), 0, hd)).astype(BF16)
    wq_p[:, 512:1024] = _mm(wqkv[:, 512:1152],
                            _onehot((640, 512), 0, lambda j: hd(j) + 64)).astype(BF16)
    wq_p[:, 1024:1536] = _mm(wqkv[:, 1152:1728], _onehot((576, 512), 0, hd)).astype(BF16)
    wq_p[:, 1536:1664] = _mm(wqkv[:, 0:640], _onehot(
        (640, 128), 0, lambda j: jnp.where(j < 64, hd(j) + 16, -1))).astype(BF16)
    wq_p[:, 1664:1792] = _mm(wqkv[:, 512:1728], _onehot(
        (1216, 128), 0,
        lambda j: hd(j & 63) + 16 + jnp.where(j < 64, 64, 640))).astype(BF16)
    cps[2].wait()
    wo_p[...] = _mm(_onehot((640, 576), 1, lambda j: jnp.where(
        j < 512, hd(j), jnp.where(j < 576, -1, hd(j & 63) + 16))), wo[...]).astype(BF16)
    bias[...] = jnp.broadcast_to(b_ref[...].astype(F32), (128, S)).T

    scale = DH ** -0.5

    def attn(x, r0):
        qkv = _mm(_ln(x).astype(BF16), wq_p[...])
        t = lambda i: qkv[:, i * 128:(i + 1) * 128]
        for c in range(8):
            kv[c, HALO:, :] = t(4 + c)
        kv[8, HALO:, :] = t(13)
        q = [t(0), t(1), t(2), t(3), t(12)]
        ks, vs = [0, 1, 2, 3, 8], [4, 5, 6, 7, 8]
        row = r0 + lax.broadcasted_iota(jnp.int32, (TM, 128), 0)
        ls = []
        for w in range(W):
            sl = pl.ds(HALO - DIL * w, TM)
            p = q[0] * kv[0, sl, :]
            for c in range(1, 5):
                p = p + q[c] * kv[ks[c], sl, :]
            p = p + pltpu.roll(p, 64, 1)
            p = p + pltpu.roll(p, 32, 1)
            if w:
                p = jnp.where(row >= DIL * w, p, -1e9 / scale)
            ls.append(p)
        m = ls[0]
        for l in ls[1:]:
            m = jnp.maximum(m, l)
        es = [jnp.exp((l - m) * scale) for l in ls]
        den = es[0]
        for e in es[1:]:
            den = den + e
        inv = 1.0 / den
        o = []
        for c in range(5):
            a = es[0] * kv[vs[c], pl.ds(HALO, TM), :]
            for w in range(1, W):
                a = a + es[w] * kv[vs[c], pl.ds(HALO - DIL * w, TM), :]
            o.append((a * inv).astype(BF16))
        kv[:, 0:HALO, :] = kv[:, TM:TM + HALO, :]
        return x + _mm(jnp.concatenate(o, axis=1), wo_p[...])

    def mlp_in(x, rows, z2):
        xn = _ln(x).astype(BF16)
        z1[rows, :] = _gelu(_mm(xn, win[:, :FH])).astype(BF16)
        z2[rows, :] = _ln(_gelu(_mm(xn, win[:, FH:]))).astype(BF16)

    def mlp_out(rows, z2):
        g = _mm(wsp[rows, :], z2[...])
        b = bias[rows, :]
        b = jnp.concatenate([b] * (FH // 128), axis=1)
        h = (z1[rows, :].astype(F32) * (g + b)).astype(BF16)
        return xs[rows, :] + _mm(h, wout[...])

    def rows_of(i):
        r0 = pl.multiple_of(i * TM, TM)
        return r0, pl.ds(r0, TM)

    cps[1].wait()
    cps[3].wait()
    kv[:, 0:HALO, :] = jnp.zeros((9, HALO, 128), F32)

    @pl.loop(0, NT)
    def _(i):
        r0, rows = rows_of(i)
        x = attn(x0[rows, :].astype(F32), r0)
        xs[rows, :] = x
        mlp_in(x, rows, z2a)

    cps[4].wait()
    cps[5].wait()
    kv[:, 0:HALO, :] = jnp.zeros((9, HALO, 128), F32)

    @pl.loop(0, NT)
    def _(i):
        r0, rows = rows_of(i)
        x = attn(mlp_out(rows, z2a), r0)
        xs[rows, :] = x
        mlp_in(x, rows, z2b)

    def out_cp(rows):
        return pltpu.make_async_copy(obuf.at[rows], o_hbm.at[rows], osem)

    @pl.loop(0, NT)
    def _(i):
        r0, rows = rows_of(i)
        obuf[rows, :] = mlp_out(rows, z2b).astype(BF16)
        out_cp(rows).start()

    pltpu.make_async_copy(obuf, o_hbm, osem).wait()


@jax.jit
def pallas_interleave_layers__sliding_local_dilated__mixer_gmlp__prompt_kernel(
    A_x, A_wqkv, A_wo, B_x, B_w_in, B_w_sp, B_b_sp, B_w_out,
):
    del B_x
    hbm = pl.BlockSpec(memory_space=pl.ANY)
    v = pltpu.VMEM
    out = pl.pallas_call(
        _kernel,
        in_specs=[hbm, hbm, hbm, hbm, hbm, pl.BlockSpec(memory_space=pltpu.VMEM), hbm],
        out_specs=hbm,
        out_shape=jax.ShapeDtypeStruct((S, D), BF16),
        scratch_shapes=[
            v((S, D), BF16), v((D, 3 * D), BF16), v((D, D), BF16), v((D, 2 * FH), BF16),
            v((S, S), BF16), v((FH, D), BF16), v((D, 1792), BF16), v((640, D), BF16),
            v((S, D), F32), v((S, FH), BF16), v((S, FH), BF16), v((S, FH), BF16),
            v((9, HALO + TM, 128), F32), v((S, 128), F32), v((S, D), BF16),
            pltpu.SemaphoreType.DMA((6,)), pltpu.SemaphoreType.DMA(()),
        ],
        compiler_params=pltpu.CompilerParams(vmem_limit_bytes=110 * 1024 * 1024),
    )(A_x.reshape(S, D), A_wqkv, A_wo, B_w_in, B_w_sp, B_b_sp.reshape(1, S), B_w_out)
    return out.reshape(1, S, D)
```

```python
import math

import jax
import jax.numpy as jnp
from jax import lax
import jax.experimental.pallas as pl
import jax.experimental.pallas.tpu as pltpu

S, D, H, DH, W, DIL = 2048, 576, 32, 18, 8, 2
FH = 2304
TM = 256
HALO = 16
NT = S // TM
F32, BF16 = jnp.float32, jnp.bfloat16


def _mm(a, b):
    return jnp.dot(a, b, preferred_element_type=F32)


def _mm_nt(a, b):
    return lax.dot_general(a, b, (((1,), (1,)), ((), ())), preferred_element_type=F32)


def _mm_tn(a, b):
    return lax.dot_general(a, b, (((0,), (0,)), ((), ())), preferred_element_type=F32)


def _ln(x):
    m = jnp.mean(x, axis=0, keepdims=True)
    c = x - m
    v = jnp.mean(c * c, axis=0, keepdims=True)
    return c * lax.rsqrt(v + 1e-5)


def _gelu(x):
    k = math.sqrt(2.0 / math.pi)
    u = x * (k + (k * 0.044715) * (x * x))
    hx = 0.5 * x
    return hx + hx * jnp.tanh(u)


def _onehot(shape, src_axis, src_fn):
    s = lax.broadcasted_iota(jnp.int32, shape, src_axis)
    d = lax.broadcasted_iota(jnp.int32, shape, 1 - src_axis)
    return jnp.where(s == src_fn(d), 1.0, 0.0).astype(BF16)


def _kernel(x_hbm, wqkv_hbm, wo_hbm, win_hbm, wsp_hbm, b_ref, wout_hbm, o_hbm,
            x0, wqkv, wo, win, wsp, wout, wq_p, wo_p, xs, z1, z2a, z2b, kv, wint,
            obuf, sems, osem):
    cps = [pltpu.make_async_copy(s, d, sems.at[i]) for i, (s, d) in enumerate(
        [(wqkv_hbm, wqkv), (x_hbm, x0), (wo_hbm, wo), (win_hbm, win),
         (wsp_hbm, wsp), (wout_hbm, wout)])]
    for c in cps:
        c.start()

    hd = lambda j: (j & 31) * DH + (j >> 5)
    cps[0].wait()
    wq_p[:, 0:512] = _mm(wqkv[:, 0:640], _onehot((640, 512), 0, hd)).astype(BF16)
    wq_p[:, 512:1024] = _mm(wqkv[:, 512:1152],
                            _onehot((640, 512), 0, lambda j: hd(j) + 64)).astype(BF16)
    wq_p[:, 1024:1536] = _mm(wqkv[:, 1152:1728], _onehot((576, 512), 0, hd)).astype(BF16)
    wq_p[:, 1536:1664] = _mm(wqkv[:, 0:640], _onehot(
        (640, 128), 0, lambda j: jnp.where(j < 64, hd(j) + 16, -1))).astype(BF16)
    wq_p[:, 1664:1792] = _mm(wqkv[:, 512:1728], _onehot(
        (1216, 128), 0,
        lambda j: hd(j & 63) + 16 + jnp.where(j < 64, 64, 640))).astype(BF16)
    cps[2].wait()
    wo_p[...] = _mm_tn(wo[...], _onehot((576, 640), 0, lambda j: jnp.where(
        j < 512, hd(j), jnp.where(j < 576, -1, hd(j & 63) + 16)))).astype(BF16)

    scale = DH ** -0.5

    def attn(x, r0):
        qkv = _mm(_ln(x).T.astype(BF16), wq_p[...])
        t = lambda i: qkv[:, i * 128:(i + 1) * 128]
        for c in range(8):
            kv[c, HALO:, :] = t(4 + c)
        kv[8, HALO:, :] = t(13)
        q = [t(0), t(1), t(2), t(3), t(12)]
        ks, vs = [0, 1, 2, 3, 8], [4, 5, 6, 7, 8]
        row = r0 + lax.broadcasted_iota(jnp.int32, (TM, 128), 0)
        ls = []
        for w in range(W):
            sl = pl.ds(HALO - DIL * w, TM)
            p = q[0] * kv[0, sl, :]
            for c in range(1, 5):
                p = p + q[c] * kv[ks[c], sl, :]
            p = p + pltpu.roll(p, 64, 1)
            p = p + pltpu.roll(p, 32, 1)
            if w:
                p = jnp.where(row >= DIL * w, p, -1e9 / scale)
            ls.append(p)
        m = ls[0]
        for l in ls[1:]:
            m = jnp.maximum(m, l)
        es = [jnp.exp((l - m) * scale) for l in ls]
        den = es[0]
        for e in es[1:]:
            den = den + e
        inv = 1.0 / den
        o = []
        for c in range(5):
            a = es[0] * kv[vs[c], pl.ds(HALO, TM), :]
            for w in range(1, W):
                a = a + es[w] * kv[vs[c], pl.ds(HALO - DIL * w, TM), :]
            o.append((a * inv).astype(BF16))
        kv[:, 0:HALO, :] = kv[:, TM:TM + HALO, :]
        return x + _mm_nt(wo_p[...], jnp.concatenate(o, axis=1))

    def mlp_in(x, rows, z2):
        xn = _ln(x).astype(BF16)
        z1[:, rows] = _gelu(_mm(wint[:FH, :], xn)).astype(BF16)
        z2[:, rows] = _ln(_gelu(_mm(wint[FH:, :], xn))).astype(BF16)

    def mlp_out(rows, z2):
        g = _mm_nt(z2[...], wsp[rows, :])
        h = (z1[:, rows].astype(F32) * (g + b_ref[:, rows].astype(F32))).astype(BF16)
        return xs[:, rows] + _mm(wout[...], h)

    def rows_of(i):
        r0 = pl.multiple_of(i * TM, TM)
        return r0, pl.ds(r0, TM)

    cps[1].wait()
    cps[3].wait()
    for j in range(0, 2 * FH, 512):
        wint[j:j + 512, :] = win[:, j:j + 512].astype(F32).T.astype(BF16)
    kv[:, 0:HALO, :] = jnp.zeros((9, HALO, 128), F32)

    @pl.loop(0, NT)
    def _(i):
        r0, rows = rows_of(i)
        x = attn(x0[:, rows].astype(F32), r0)
        xs[:, rows] = x
        mlp_in(x, rows, z2a)

    cps[4].wait()
    cps[5].wait()
    kv[:, 0:HALO, :] = jnp.zeros((9, HALO, 128), F32)

    @pl.loop(0, NT)
    def _(i):
        r0, rows = rows_of(i)
        x = attn(mlp_out(rows, z2a), r0)
        xs[:, rows] = x
        mlp_in(x, rows, z2b)

    def out_cp(rows):
        return pltpu.make_async_copy(obuf.at[:, rows], o_hbm.at[:, rows], osem)

    @pl.loop(0, NT)
    def _(i):
        r0, rows = rows_of(i)
        obuf[:, rows] = mlp_out(rows, z2b).astype(BF16)
        out_cp(rows).start()

    pltpu.make_async_copy(obuf, o_hbm, osem).wait()


@jax.jit
def pallas_interleave_layers__sliding_local_dilated__mixer_gmlp__prompt_kernel(
    A_x, A_wqkv, A_wo, B_x, B_w_in, B_w_sp, B_b_sp, B_w_out,
):
    del B_x
    hbm = pl.BlockSpec(memory_space=pltpu.HBM)
    v = pltpu.VMEM
    out = pl.pallas_call(
        _kernel,
        in_specs=[hbm, hbm, hbm, hbm, hbm, pl.BlockSpec(memory_space=pltpu.VMEM), hbm],
        out_specs=hbm,
        out_shape=jax.ShapeDtypeStruct((D, S), BF16),
        scratch_shapes=[
            v((D, S), BF16), v((D, 3 * D), BF16), v((D, D), BF16), v((D, 2 * FH), BF16),
            v((S, S), BF16), v((D, FH), BF16), v((D, 1792), BF16), v((D, 640), BF16),
            v((D, S), F32), v((FH, S), BF16), v((FH, S), BF16), v((FH, S), BF16),
            v((9, HALO + TM, 128), F32), v((2 * FH, D), BF16), v((D, S), BF16),
            pltpu.SemaphoreType.DMA((6,)), pltpu.SemaphoreType.DMA(()),
        ],
        compiler_params=pltpu.CompilerParams(vmem_limit_bytes=110 * 1024 * 1024),
    )(A_x.reshape(S, D).T, A_wqkv, A_wo, B_w_in, B_w_sp, B_b_sp.reshape(1, S), B_w_out.T)
    return out.T.reshape(1, S, D)
```

```python
import math

import jax
import jax.numpy as jnp
from jax import lax
import jax.experimental.pallas as pl
import jax.experimental.pallas.tpu as pltpu

S, D, H, DH, W, DIL = 2048, 576, 32, 18, 8, 2
FH = 2304
TM = 256
HALO = 16
AR, FC, GC, OC = 16, 256, 256, 192
QW, AW = 1, 60
NT = S // TM
F32, BF16 = jnp.float32, jnp.bfloat16


def _mm(a, b):
    return jnp.dot(a, b, preferred_element_type=F32)


def _mm_nt(a, b):
    return lax.dot_general(a, b, (((1,), (1,)), ((), ())), preferred_element_type=F32)


def _mm_tn(a, b):
    return lax.dot_general(a, b, (((0,), (0,)), ((), ())), preferred_element_type=F32)


def _ln(x):
    m = jnp.mean(x, axis=0, keepdims=True)
    c = x - m
    v = jnp.mean(c * c, axis=0, keepdims=True)
    return c * lax.rsqrt(v + 1e-5)


def _gelu(x):
    k = math.sqrt(2.0 / math.pi)
    u = x * (k + (k * 0.044715) * (x * x))
    hx = 0.5 * x
    return hx + hx * jnp.tanh(u)


def _onehot(shape, src_axis, src_fn):
    s = lax.broadcasted_iota(jnp.int32, shape, src_axis)
    d = lax.broadcasted_iota(jnp.int32, shape, 1 - src_axis)
    return jnp.where(s == src_fn(d), 1.0, 0.0).astype(BF16)


def _kernel(x_hbm, wqkv_hbm, wo_hbm, win_hbm, wsp_hbm, b_ref, wout_hbm, o_hbm,
            x0, wqkv, wo, win, wsp, wout, wq_p, wo_p, xs, xb, x0f, z1a, z1b, z2a, z2b, kv, wint,
            obuf, ob, zt, hb, wt, sems, osem):
    cps = [pltpu.make_async_copy(s, d, sems.at[i]) for i, (s, d) in enumerate(
        [(wqkv_hbm, wqkv), (x_hbm, x0), (wo_hbm, wo), (win_hbm, win),
         (wsp_hbm, wsp), (wout_hbm, wout)])]
    for c in cps[:4]:
        c.start()

    hd = lambda j: (j & 31) * DH + (j >> 5)
    cps[0].wait()
    slabs = list(enumerate((0, 128, 256, 384, 448)))
    wq_p[1600:1664, :] = jnp.zeros((64, D), BF16)
    for k, l in slabs:
        wt[k, 0:1664, :] = wqkv[l:l + 128, 0:1664].astype(F32).T
        wt[k, 1600:1728, :] = wqkv[l:l + 128, 1600:1728].astype(F32).T
        for c in range(3):
            for d in range(DH):
                o = c * 512 + d * 32 if d < 16 else (1536, 1664, 1728)[c] + (d - 16) * 32
                wq_p[o:o + 32, l:l + 128] = wt[
                    k, pl.ds(c * D + d, H, stride=DH), :].astype(BF16)
    cps[2].wait()
    for k, l in slabs:
        wt[k, 0:D, :] = wo[:, l:l + 128].astype(F32)
        wt[k, 1152:1216, :] = jnp.zeros((64, 128), F32)
        for d in range(DH):
            o = 640 + d * 32 + (64 if d >= 16 else 0)
            wt[k, o:o + 32, :] = wt[k, pl.ds(d, H, stride=DH), :]
        wo_p[l:l + 128, :] = wt[k, 640:1280, :].T.astype(BF16)

    scale = DH ** -0.5

    def g_attn(i, src, dst):
        r0, rows = rows_of(i)
        xn = _ln(src[:, rows].astype(F32)).T.astype(BF16)
        yield 4
        for c0 in range(0, 14, 2):
            y = _mm_nt(xn, wq_p[c0 * 128:(c0 + 2) * 128, :])
            kv[c0, HALO:, :] = y[:, :128]
            kv[c0 + 1, HALO:, :] = y[:, 128:]
            yield QW
        qs, ks, vs = [0, 1, 2, 3, 12], [4, 5, 6, 7, 13], [8, 9, 10, 11, 13]
        for a0 in range(0, TM, AR):
            q = [kv[c, pl.ds(HALO + a0, AR), :] for c in qs]
            row = r0 + a0 + lax.broadcasted_iota(jnp.int32, (AR, 128), 0)
            ls = []
            for w in range(W):
                sl = pl.ds(HALO + a0 - DIL * w, AR)
                p = q[0] * kv[ks[0], sl, :]
                for c in range(1, 5):
                    p = p + q[c] * kv[ks[c], sl, :]
                p = p + pltpu.roll(p, 64, 1)
                p = p + pltpu.roll(p, 32, 1)
                if w and a0 < DIL * w:
                    p = jnp.where(row >= DIL * w, p, -1e9 / scale)
                ls.append(p)
            m = ls[0]
            for l in ls[1:]:
                m = jnp.maximum(m, l)
            es = [jnp.exp((l - m) * scale) for l in ls]
            den = es[0]
            for e in es[1:]:
                den = den + e
            inv = 1.0 / den
            for c in range(5):
                a = es[0] * kv[vs[c], pl.ds(HALO + a0, AR), :]
                for w in range(1, W):
                    a = a + es[w] * kv[vs[c], pl.ds(HALO + a0 - DIL * w, AR), :]
                ob[a0:a0 + AR, c * 128:(c + 1) * 128] = (a * inv).astype(BF16)
            yield AW * AR / TM
        kv[4:, 0:HALO, :] = kv[4:, TM:TM + HALO, :]
        for d0 in range(0, D, 192):
            ds = slice(d0, d0 + 192)
            dst[ds, rows] = src[ds, rows].astype(F32) + _mm_nt(wo_p[ds, :], ob[...])
            yield QW

    def g_in(i, src, z1, z2):
        rows = rows_of(i)[1]
        xn = _ln(src[:, rows]).astype(BF16)
        yield 1
        tot = 0.0
        for f0 in range(0, FH, FC):
            z = _gelu(_mm(wint[FH + f0:FH + f0 + FC, :], xn))
            zt[f0:f0 + FC, :] = z
            tot = tot + z.reshape(FC // 8, 8, TM).sum(0)
            yield 1
        m = jnp.sum(tot, axis=0, keepdims=True) * (1.0 / FH)
        tot = 0.0
        n = FH // FC
        half = n // 2
        for j in range(n):
            f0 = j * FC
            z1[f0:f0 + FC, rows] = _gelu(_mm(wint[f0:f0 + FC, :], xn)).astype(BF16)
            yield 0.5
            if j < half:
                for e0 in range(j * n // half * FC, (j + 1) * n // half * FC, FC):
                    c = zt[e0:e0 + FC, :] - m
                    tot = tot + (c * c).reshape(FC // 8, 8, TM).sum(0)
                if j == half - 1:
                    r = lax.rsqrt(jnp.sum(tot, axis=0, keepdims=True) * (1.0 / FH) + 1e-5)
            else:
                k, nk = j - half, n - half
                for e0 in range(k * n // nk * FC, (k + 1) * n // nk * FC, FC):
                    z2[e0:e0 + FC, rows] = ((zt[e0:e0 + FC, :] - m) * r).astype(BF16)
            yield 0.5

    def g_out(i, z1, z2, src, dst, GC=GC, OC=OC):
        rows = rows_of(i)[1]
        b = b_ref[:, rows].astype(F32)
        for f0 in range(0, FH, GC):
            g = _mm_nt(z2[f0:f0 + GC, :], wsp[rows, :])
            hb[f0:f0 + GC, :] = (z1[f0:f0 + GC, rows].astype(F32) * (g + b)).astype(BF16)
            yield 288.0 * GC / FH
        for d0 in range(0, D, OC):
            ds = slice(d0, d0 + OC)
            dst[ds, rows] = (src[ds, rows] + _mm(wout[ds, :], hb[...])).astype(dst.dtype)
            yield 81.0 * OC / D

    def merge(*gs):
        done = [0.0] * len(gs)
        while min(done) < 2:
            k = done.index(min(done))
            c = next(gs[k][0], None)
            done[k] = 2 if c is None else done[k] + c / gs[k][1]

    def rows_of(i):
        r0 = i * TM if isinstance(i, int) else pl.multiple_of(i * TM, TM)
        return r0, pl.ds(r0, TM)

    cps[1].wait()
    kv[4:, 0:HALO, :] = jnp.zeros((10, HALO, 128), F32)

    t_attn = lambda i, src, dst: (g_attn(i, src, dst), 4 + 10 * QW + AW)
    t_in = lambda i, src, z1, z2: (g_in(i, src, z1, z2), 1 + 2 * FH // FC)
    t_out = lambda i: (g_out(i, z1a, z2a, xs, xb), 369)

    with jax.named_scope('ph_0'):
        merge(t_attn(0, x0, xs))
        cps[3].wait()
        for c in cps[4:]:
            c.start()
        for j in range(0, 2 * FH, 512):
            wint[j:j + 512, :] = win[:, j:j + 512].astype(F32).T.astype(BF16)

        @pl.loop(0, NT - 1)
        def _(i):
            merge(t_in(i, xs, z1a, z2a), t_attn(i + 1, x0, xs))

        merge(t_in(NT - 1, xs, z1a, z2a))

    cps[4].wait()
    cps[5].wait()
    kv[4:, 0:HALO, :] = jnp.zeros((10, HALO, 128), F32)

    with jax.named_scope('ph_1'):
        merge(t_out(0))
        merge(t_out(1), t_attn(0, xb, x0f))

        @pl.loop(0, NT - 2)
        def _(i):
            merge(t_out(i + 2), t_in(i, x0f, z1b, z2b), t_attn(i + 1, xb, x0f))

        merge(t_in(NT - 2, x0f, z1b, z2b), t_attn(NT - 1, xb, x0f))
        merge(t_in(NT - 1, x0f, z1b, z2b))

    def out_cp(rows):
        return pltpu.make_async_copy(obuf.at[:, rows], o_hbm.at[:, rows], osem)

    with jax.named_scope('ph_2'):
        @pl.loop(0, NT)
        def _(i):
            merge((g_out(i, z1b, z2b, x0f, obuf, FH, D), 369))
            out_cp(rows_of(i)[1]).start()

    pltpu.make_async_copy(obuf, o_hbm, osem).wait()


@jax.jit
def pallas_interleave_layers__sliding_local_dilated__mixer_gmlp__prompt_kernel(
    A_x, A_wqkv, A_wo, B_x, B_w_in, B_w_sp, B_b_sp, B_w_out,
):
    del B_x
    hbm = pl.BlockSpec(memory_space=pltpu.HBM)
    v = pltpu.VMEM
    out = pl.pallas_call(
        _kernel,
        in_specs=[hbm, hbm, hbm, hbm, hbm, pl.BlockSpec(memory_space=pltpu.VMEM), hbm],
        out_specs=hbm,
        out_shape=jax.ShapeDtypeStruct((D, S), BF16),
        scratch_shapes=[
            v((D, S), BF16), v((D, 3 * D), BF16), v((D, D), BF16), v((D, 2 * FH), BF16),
            v((S, S), BF16), v((D, FH), BF16), v((1792, D), BF16), v((D, 640), BF16),
            v((D, S), F32), v((D, S), F32), v((D, S), F32), v((FH, S), BF16), v((FH, S), BF16), v((FH, S), BF16), v((FH, S), BF16),
            v((14, HALO + TM, 128), F32), v((2 * FH, D), BF16), v((D, S), BF16),
            v((TM, 640), BF16), v((FH, TM), F32), v((FH, TM), BF16), v((5, 3 * D, 128), F32),
            pltpu.SemaphoreType.DMA((6,)), pltpu.SemaphoreType.DMA(()),
        ],
        compiler_params=pltpu.CompilerParams(vmem_limit_bytes=120 * 1024 * 1024),
    )(A_x.reshape(S, D).T, A_wqkv, A_wo, B_w_in, B_w_sp, B_b_sp.reshape(1, S), B_w_out.T)
    return out.T.reshape(1, S, D)
```
